```python
import jax
import jax.numpy as jnp

def _softmax(x, axis=-1):
    return jax.nn.softmax(x, axis=axis)

def _gelu(x):
    return jax.nn.gelu(x, approximate=True)

def _silu(x):
    return jax.nn.silu(x)

def _sigmoid(x):
    return jax.nn.sigmoid(x)

def _layernorm(x, axis=-1, eps=1e-05):
    m = jnp.mean(x, axis=axis, keepdims=True)
    v = jnp.var(x, axis=axis, keepdims=True)
    return (x - m) / jnp.sqrt(v + eps)

def _scatter_add(tgt, idx, src, axis=0):
    return tgt.at[idx].add(src)

def _segment_sum(src, seg, n):
    return jax.ops.segment_sum(src, seg, n)

class _Rng:

    def __init__(self, key):
        self._k = key

    def _next(self):
        self._k, sub = jax.random.split(self._k)
        return sub

    def normal(self, shape):
        return jax.random.normal(self._next(), shape, dtype=jnp.bfloat16)

    def randint(self, lo, hi, shape):
        return jax.random.randint(self._next(), shape, lo, hi, dtype=jnp.int32)

    def uniform(self, shape, lo=0.0, hi=1.0):
        return jax.random.uniform(self._next(), shape, jnp.bfloat16, lo, hi)

    def permutation(self, n):
        return jax.random.permutation(self._next(), n)
kernel_name = 'recurrent_scan__memory_aug_recurrent_mem_tr__glu_gated_glu__prompt'

def setup_inputs():
    _rng = _Rng(jax.random.key(int.from_bytes(__import__("os").urandom(4), "little")))
    _w = lambda a: (lambda t: t.astype(jnp.bfloat16) if jnp.issubdtype(t.dtype, jnp.floating) else t)(jnp.asarray(a))

    def _A_setup():
        B, S, Dm = (1, 2048, 1024)
        H, Dh = (32, 128)
        M, seg = (8, 32)
        seg = min(seg, S)
        S = S // seg * seg
        return {'x': _w((lambda *s: _rng.normal(s) * 0.05)(B, S, Dm)), 'mem0': _w((lambda *s: _rng.normal(s) * 0.05)(B, M, Dm)), 'Wq': _w((lambda *s: _rng.normal(s) * 0.05)(Dm, H, Dh) * Dm ** (-0.5)), 'Wk': _w((lambda *s: _rng.normal(s) * 0.05)(Dm, H, Dh) * Dm ** (-0.5)), 'Wv': _w((lambda *s: _rng.normal(s) * 0.05)(Dm, H, Dh) * Dm ** (-0.5)), 'Wo': _w((lambda *s: _rng.normal(s) * 0.05)(H, Dh, Dm) * (H * Dh) ** (-0.5)), 'seg_len': seg}
    _A_in = _A_setup()

    def _B_setup():
        B, S, D, F = (1, 2048, 1024, 3584)
        return {'x': _w((lambda *s: _rng.normal(s) * 0.05)(B, S, D)), 'w_gate': _w((lambda *s: _rng.normal(s) * 0.05)(D, F)), 'w_up': _w((lambda *s: _rng.normal(s) * 0.05)(D, F)), 'w_down': _w((lambda *s: _rng.normal(s) * 0.05)(F, D))}
    _B_in = _B_setup()
    return {'A_x': _A_in['x'], 'A_mem0': _A_in['mem0'], 'A_Wq': _A_in['Wq'], 'A_Wk': _A_in['Wk'], 'A_Wv': _A_in['Wv'], 'A_Wo': _A_in['Wo'], 'A_seg_len': _A_in['seg_len'], 'B_x': _B_in['x'], 'B_w_gate': _B_in['w_gate'], 'B_w_up': _B_in['w_up'], 'B_w_down': _B_in['w_down']}

def reference(A_x, A_mem0, A_Wq, A_Wk, A_Wv, A_Wo, A_seg_len, B_x, B_w_gate, B_w_up, B_w_down):

    def _A_ref(x, mem0, Wq, Wk, Wv, Wo, seg_len):
        B, S, Dm = x.shape
        H, Dh = (Wq.shape[1], Wq.shape[2])
        M = mem0.shape[1]
        scale = Dh ** (-0.5)
        n_seg = S // seg_len
        L = M + seg_len
        idx = jnp.arange(L)
        mask = (idx[:, None] < M) | (idx[:, None] >= idx[None, :])
        mem = mem0
        outs = []
        for s in range(n_seg):
            xs = x[:, s * seg_len:(s + 1) * seg_len, :].copy()
            h = jnp.concatenate([mem, xs], axis=1)
            q = jnp.einsum('btd,dhe->bhte', h, Wq)
            k = jnp.einsum('btd,dhe->bhte', h, Wk)
            v = jnp.einsum('btd,dhe->bhte', h, Wv)
            scores = jnp.einsum('bhqe,bhke->bhqk', q, k) * scale
            scores = jnp.where(mask[None, None], scores, -1000000000.0)
            p = _softmax(scores, axis=-1)
            o = jnp.einsum('bhqk,bhke->bhqe', p, v)
            o = jnp.einsum('bhte,hed->btd', o, Wo)
            mem = o[:, :M, :].copy()
            outs.append(o[:, M:, :])
        return jnp.concatenate(outs, axis=1)

    def _B_ref(x, w_gate, w_up, w_down):
        g = jnp.einsum('bsd,df->bsf', x, w_gate)
        u = jnp.einsum('bsd,df->bsf', x, w_up)
        h = _sigmoid(g) * u
        return jnp.einsum('bsf,fd->bsd', h, w_down)
    x = A_x
    xn = _layernorm(x, axis=-1)
    s = _A_ref(xn, A_mem0, A_Wq, A_Wk, A_Wv, A_Wo, A_seg_len)
    g = _silu(_B_ref(xn, B_w_gate, B_w_up, B_w_down))
    return x + s * g
```

```python
import functools
import jax, jax.numpy as jnp, numpy as np
from jax import lax
from jax.experimental import pallas as pl
from jax.experimental.pallas import tpu as pltpu

S, D, H, E, M, F = 2048, 1024, 32, 128, 8, 3584
SEG = 32
NSEG = S // SEG
L = M + SEG
FC = 512
NFC = F // FC
RB = 512
PD = 128
NP = D // PD
HG = 4

def kernel(x_hbm, mem_ref, wq_hbm, wk_hbm, wv_hbm, wo_hbm, wg_hbm, wu_hbm, wd_hbm,
           out_hbm,
           x_v, xn_v, acc_v, out_v, wqkv, wo_v, raw3, rawo, wg_v, wu_v, wd_v, o_v,
           sem_x, sem_glu, sem_raw, sem_out):
    f32, bf16, u32 = jnp.float32, jnp.bfloat16, jnp.uint32

    def glu_copies(c, slot):
        c0 = pl.multiple_of(c * FC, FC)
        return (pltpu.make_async_copy(wg_hbm.at[:, pl.ds(c0, FC)], wg_v.at[slot], sem_glu.at[slot, 0]),
                pltpu.make_async_copy(wu_hbm.at[:, pl.ds(c0, FC)], wu_v.at[slot], sem_glu.at[slot, 1]),
                pltpu.make_async_copy(wd_hbm.at[pl.ds(c0, FC), :], wd_v.at[slot], sem_glu.at[slot, 2]))

    def raw_copies(p, slot):
        d0 = pl.multiple_of(p * PD, PD)
        h0 = pl.multiple_of(p * (H // NP), H // NP)
        return (pltpu.make_async_copy(wq_hbm.at[pl.ds(d0, PD)], raw3.at[slot, 0], sem_raw.at[slot, 0]),
                pltpu.make_async_copy(wk_hbm.at[pl.ds(d0, PD)], raw3.at[slot, 1], sem_raw.at[slot, 1]),
                pltpu.make_async_copy(wv_hbm.at[pl.ds(d0, PD)], raw3.at[slot, 2], sem_raw.at[slot, 2]),
                pltpu.make_async_copy(wo_hbm.at[pl.ds(h0, H // NP)], rawo.at[slot], sem_raw.at[slot, 3]))

    xcp = pltpu.make_async_copy(x_hbm, x_v, sem_x)
    xcp.start()
    for cp in glu_copies(0, 0): cp.start()
    for cp in raw_copies(0, 0): cp.start()
    for cp in glu_copies(1, 1): cp.start()
    for cp in raw_copies(1, 1): cp.start()
    xcp.wait()

    def ln_body(i, _):
        r0 = pl.multiple_of(i * 128, 128)
        xv = x_v[pl.ds(r0, 128), :].astype(f32)
        mu = jnp.mean(xv, axis=-1, keepdims=True)
        xc = xv - mu
        var = jnp.mean(xc * xc, axis=-1, keepdims=True)
        xn_v[pl.ds(r0, 128), :] = (xc * lax.rsqrt(var + 1e-5)).astype(bf16)
        return None
    lax.fori_loop(0, S // 128, ln_body, None)

    def relayout(p, slot):
        for m in range(3):
            def body(i, _):
                r0 = pl.multiple_of(i * 16, 16)
                v = raw3[slot, m, pl.ds(r0, 16)]
                u = pltpu.bitcast(v, u32).reshape(8, 2, 16, E)
                a = u[:, 0]; b = u[:, 1]
                lo = (a & np.uint32(0xFFFF)) | (b << 16)
                hi = (a >> 16) | (b & np.uint32(0xFFFF0000))
                lot = jnp.transpose(lo, (1, 0, 2)); hit = jnp.transpose(hi, (1, 0, 2))
                o0 = pl.multiple_of(p * (PD // 2) + i * 8, 8)
                for hp in range(16):
                    c = m * H * E + 2 * hp * E
                    wqkv[pl.ds(o0, 8), c:c + E] = lot[hp]
                    wqkv[pl.ds(o0, 8), c + E:c + 2 * E] = hit[hp]
                return None
            lax.fori_loop(0, PD // 16, body, None)
        nh = H // NP
        for j in range(nh):
            o0 = pl.multiple_of((p * nh + j) * (E // 2), E // 2)
            wo_v[pl.ds(o0, E // 2), :] = pltpu.bitcast(rawo[slot, j], u32)

    def glu_body(c, _):
        slot = c % 2
        for cp in raw_copies(c, slot): cp.wait()
        @pl.when(c < NFC)
        def _():
            for cp in glu_copies(c, slot): cp.wait()
            def rows(r, _):
                r0 = pl.multiple_of(r * RB, RB)
                xb = xn_v[pl.ds(r0, RB), :]
                g = jnp.dot(xb, wg_v[slot], preferred_element_type=f32)
                u = jnp.dot(xb, wu_v[slot], preferred_element_type=f32)
                hh = (u / (1.0 + jnp.exp(-g))).astype(bf16)
                d = jnp.dot(hh, wd_v[slot], preferred_element_type=f32)
                @pl.when(c == 0)
                def _():
                    acc_v[pl.ds(r0, RB), :] = d
                @pl.when(c > 0)
                def _():
                    acc_v[pl.ds(r0, RB), :] += d
                return None
            lax.fori_loop(0, S // RB, rows, None)
        relayout(c, slot)
        @pl.when(c + 2 < NFC)
        def _():
            for cp in glu_copies(c + 2, slot): cp.start()
        @pl.when(c + 2 < NP)
        def _():
            for cp in raw_copies(c + 2, slot): cp.start()
        return None
    lax.fori_loop(0, NP, glu_body, None)

    row = lax.broadcasted_iota(jnp.int32, (L, L), 0)
    col = lax.broadcasted_iota(jnp.int32, (L, L), 1)
    mask = (row < M) | (row >= col)
    scale = E ** -0.5
    OB = 256
    def out_copy(b):
        r0 = pl.multiple_of(b * OB, OB)
        return pltpu.make_async_copy(out_v.at[pl.ds(r0, OB)], out_hbm.at[pl.ds(r0, OB)], sem_out.at[b])

    def step(s, mem):
        r0 = pl.multiple_of(s * SEG, SEG)
        xs = xn_v[pl.ds(r0, SEG), :].astype(f32)
        hf = jnp.concatenate([mem, xs], axis=0)
        for g in range(H // HG):
            def proj(m):
                c = m * H * E + g * HG * E
                w = pltpu.bitcast(wqkv[:, c:c + HG * E], bf16)
                return jnp.dot(hf, w, preferred_element_type=f32)
            q = proj(0); k = proj(1); v = proj(2)
            for j in range(HG):
                qh = q[:, j * E:(j + 1) * E]; kh = k[:, j * E:(j + 1) * E]; vh = v[:, j * E:(j + 1) * E]
                sc = lax.dot_general(qh, kh, (((1,), (1,)), ((), ())), preferred_element_type=f32) * scale
                sc = jnp.where(mask, sc, -1e9)
                mx = jnp.max(sc, axis=-1, keepdims=True)
                p = jnp.exp(sc - mx)
                p = p / jnp.sum(p, axis=-1, keepdims=True)
                o = jnp.dot(p, vh, preferred_element_type=f32)
                hh = g * HG + j
                o_v[:, hh * E:(hh + 1) * E] = o
        wo = pltpu.bitcast(wo_v[...], bf16)
        res = jnp.dot(o_v[...], wo, preferred_element_type=f32)
        st = res[M:].astype(bf16).astype(f32)
        gl = acc_v[pl.ds(r0, SEG), :].astype(bf16).astype(f32)
        gl = gl / (1.0 + jnp.exp(-gl))
        out_v[pl.ds(r0, SEG), :] = (x_v[pl.ds(r0, SEG), :].astype(f32) + st * gl).astype(bf16)
        @pl.when((s + 1) % (OB // SEG) == 0)
        def _():
            out_copy(s // (OB // SEG)).start()
        return res[:M].astype(bf16).astype(f32)
    lax.fori_loop(0, NSEG, step, mem_ref[...].astype(f32))
    for b in range(S // OB):
        out_copy(b).wait()


@functools.partial(jax.jit, static_argnames=("A_seg_len",))
def pallas_recurrent_scan__memory_aug_recurrent_mem_tr__glu_gated_glu__prompt_kernel(A_x, A_mem0, A_Wq, A_Wk, A_Wv, A_Wo, A_seg_len, B_x, B_w_gate, B_w_up, B_w_down):
    f32, bf16, u32 = jnp.float32, jnp.bfloat16, jnp.uint32
    hbm = pl.BlockSpec(memory_space=pl.ANY)
    vm = pl.BlockSpec(memory_space=pltpu.VMEM)
    V = pltpu.VMEM
    out = pl.pallas_call(
        kernel,
        out_shape=jax.ShapeDtypeStruct((S, D), bf16),
        in_specs=[hbm, vm, hbm, hbm, hbm, hbm, hbm, hbm, hbm],
        out_specs=hbm,
        scratch_shapes=[
            V((S, D), bf16), V((S, D), bf16), V((S, D), f32), V((S, D), bf16),
            V((D // 2, 3 * H * E), u32), V((H * E // 2, D), u32),
            V((2, 3, PD, H, E), bf16), V((2, H // NP, E, D), bf16),
            V((2, D, FC), bf16), V((2, D, FC), bf16), V((2, FC, D), bf16),
            V((L, H * E), f32),
            pltpu.SemaphoreType.DMA(()), pltpu.SemaphoreType.DMA((2, 3)),
            pltpu.SemaphoreType.DMA((2, 4)), pltpu.SemaphoreType.DMA((S // 256,)),
        ],
        compiler_params=pltpu.CompilerParams(vmem_limit_bytes=110 * 1024 * 1024),
    )(A_x.reshape(S, D), A_mem0.reshape(M, D), A_Wq, A_Wk, A_Wv, A_Wo, B_w_gate, B_w_up, B_w_down)
    return out.reshape(1, S, D)
```

```python
import functools
import jax, jax.numpy as jnp, numpy as np
from jax import lax
from jax.experimental import pallas as pl
from jax.experimental.pallas import tpu as pltpu

S, D, H, E, M, F = 2048, 1024, 32, 128, 8, 3584
SEG = 32
NSEG = S // SEG
L = M + SEG
FC = 512
NFC = F // FC
RB = 1024
NB = S // RB
PD = 128
NP = D // PD
HG = 16

def kernel(x_hbm, mem_ref, wq_hbm, wk_hbm, wv_hbm, wo_hbm, wg_hbm, wu_hbm, wd_hbm,
           out_hbm,
           x_v, xn_v, acc_v, out_v, wqkv, wo_v, raw3, rawo, wg_v, wu_v, wd_v, o_v,
           sem_x, sem_glu, sem_raw, sem_out):
    f32, bf16, u32 = jnp.float32, jnp.bfloat16, jnp.uint32

    def glu_copies(c, slot):
        c0 = pl.multiple_of(c * FC, FC)
        return (pltpu.make_async_copy(wg_hbm.at[:, pl.ds(c0, FC)], wg_v.at[slot, :, pl.ds(0, FC)], sem_glu.at[slot, 0]),
                pltpu.make_async_copy(wu_hbm.at[:, pl.ds(c0, FC)], wg_v.at[slot, :, pl.ds(FC, FC)], sem_glu.at[slot, 1]),
                pltpu.make_async_copy(wd_hbm.at[pl.ds(c0, FC), :], wd_v.at[slot], sem_glu.at[slot, 2]))

    def raw_copies(p, slot):
        d0 = pl.multiple_of(p * PD, PD)
        h0 = pl.multiple_of(p * (H // NP), H // NP)
        return (pltpu.make_async_copy(wq_hbm.at[pl.ds(d0, PD)], raw3.at[slot, 0], sem_raw.at[slot, 0]),
                pltpu.make_async_copy(wk_hbm.at[pl.ds(d0, PD)], raw3.at[slot, 1], sem_raw.at[slot, 1]),
                pltpu.make_async_copy(wv_hbm.at[pl.ds(d0, PD)], raw3.at[slot, 2], sem_raw.at[slot, 2]),
                pltpu.make_async_copy(wo_hbm.at[pl.ds(pl.multiple_of(p * (H // NP) * E, (H // NP) * E), H // NP * E)], rawo.at[slot], sem_raw.at[slot, 3]))

    NX = 4
    XR = S // NX
    xcps = [pltpu.make_async_copy(x_hbm.at[pl.ds(i * XR, XR)], x_v.at[pl.ds(i * XR, XR)], sem_x.at[i]) for i in range(NX)]
    for cp in xcps: cp.start()
    for cp in glu_copies(0, 0): cp.start()
    acc_v[...] = jnp.zeros_like(acc_v)
    raw3[2] = jnp.zeros_like(raw3[2])
    rawo[2] = jnp.zeros_like(rawo[2])

    def ln_body(i, _):
        r0 = pl.multiple_of(i * 128, 128)
        xv = x_v[pl.ds(r0, 128), :].astype(f32)
        mu = jnp.mean(xv, axis=-1, keepdims=True)
        xc = xv - mu
        var = jnp.mean(xc * xc, axis=-1, keepdims=True)
        xn_v[pl.ds(pl.multiple_of(r0 // 2, 64), 64), :] = pltpu.bitcast((xc * lax.rsqrt(var + 1e-5)).astype(bf16), u32)
        return None
    for i in range(NX):
        xcps[i].wait()
        if i == NX - 1:
            for cp in raw_copies(0, 0): cp.start()
        lax.fori_loop(i * (XR // 128), (i + 1) * (XR // 128), ln_body, None)
    for cp in glu_copies(1, 1): cp.start()
    for cp in raw_copies(1, 1): cp.start()

    def relayout(p, slot, r):
        for m in range(3):
            for i in range(PD // 16 // NB):
                r0 = pl.multiple_of(r * (PD // NB) + i * 16, 16)
                v = raw3[slot, m, pl.ds(r0, 16)]
                u = pltpu.bitcast(v, u32).reshape(8, 2, 16, E)
                a = u[:, 0]; b = u[:, 1]
                lo = (a & np.uint32(0xFFFF)) | (b << 16)
                hi = (a >> 16) | (b & np.uint32(0xFFFF0000))
                lot = jnp.transpose(lo, (1, 0, 2)); hit = jnp.transpose(hi, (1, 0, 2))
                o0 = pl.multiple_of(p * (PD // 2) + r * (PD // NB // 2) + i * 8, 8)
                for hp in range(16):
                    c = m * H * E + 2 * hp * E
                    wqkv[pl.ds(o0, 8), c:c + E] = lot[hp]
                    wqkv[pl.ds(o0, 8), c + E:c + 2 * E] = hit[hp]
        nr = (H // NP) * E // NB
        o0 = pl.multiple_of(p * (H // NP) * E // 2 + r * (nr // 2), nr // 2)
        wo_v[pl.ds(o0, nr // 2), :] = pltpu.bitcast(rawo[slot, pl.ds(pl.multiple_of(r * nr, nr), nr), :], u32)

    def glu_body(c, _):
        slot = c % 2
        rs = (c + 2) % 3
        p = (c + NP - 1) % NP
        @pl.when(c > 0)
        def _():
            for cp in raw_copies(c - 1, rs): cp.wait()
        @pl.when(c < NFC)
        def _():
            for cp in glu_copies(c, slot): cp.wait()
            def rows(r, _):
                r0 = pl.multiple_of(r * RB, RB)
                xb = pltpu.bitcast(xn_v[pl.ds(pl.multiple_of(r0 // 2, RB // 2), RB // 2), :], bf16)
                gu = jnp.dot(xb, wg_v[slot], preferred_element_type=f32)
                g = gu[:, :FC]; u = gu[:, FC:]
                hh = (u / (1.0 + jnp.exp(-g))).astype(bf16)
                d = jnp.dot(hh, wd_v[slot], preferred_element_type=f32)
                acc_v[pl.ds(r0, RB), :] += d
                relayout(p, rs, r)
                return None
            lax.fori_loop(0, S // RB, rows, None)
        @pl.when(c >= NFC)
        def _():
            lax.fori_loop(0, NB, lambda r, _: relayout(p, rs, r), None)
        @pl.when(c + 2 < NFC)
        def _():
            for cp in glu_copies(c + 2, slot): cp.start()
        @pl.when(c + 2 < NP)
        def _():
            for cp in raw_copies(c + 2, rs): cp.start()
        return None
    lax.fori_loop(0, NP + 1, glu_body, None)

    row = lax.broadcasted_iota(jnp.int32, (L, L), 0)
    col = lax.broadcasted_iota(jnp.int32, (L, L), 1)
    mask = (row < M) | (row >= col)
    scale = E ** -0.5
    OB = 256
    def out_copy(b):
        r0 = pl.multiple_of(b * OB, OB)
        return pltpu.make_async_copy(out_v.at[pl.ds(r0, OB)], out_hbm.at[pl.ds(r0, OB)], sem_out.at[b])

    def step(s, mem):
        r0 = pl.multiple_of(s * SEG, SEG)
        xs = pltpu.bitcast(xn_v[pl.ds(pl.multiple_of(s * (SEG // 2), SEG // 2), SEG // 2), :], bf16).astype(f32)
        hf = jnp.concatenate([mem, xs], axis=0)
        NG = H // HG
        for g in range(NG):
            def proj(m):
                c = m * H * E + g * HG * E
                w = pltpu.bitcast(wqkv[:, c:c + HG * E], bf16)
                return jnp.dot(hf, w, preferred_element_type=f32)
            q = proj(0); k = proj(1)
            scs = []
            for j in range(HG):
                qh = q[:, j * E:(j + 1) * E]; kh = k[:, j * E:(j + 1) * E]
                scs.append(lax.dot_general(qh, kh, (((1,), (1,)), ((), ())), preferred_element_type=f32))
            v = proj(2)
            for j in range(HG):
                vh = v[:, j * E:(j + 1) * E]
                sc = jnp.where(mask, scs[j] * scale, -1e9)
                mx = jnp.max(sc, axis=-1, keepdims=True)
                p = jnp.exp(sc - mx)
                p = p / jnp.sum(p, axis=-1, keepdims=True)
                o = jnp.dot(p, vh, preferred_element_type=f32)
                hh = g * HG + j
                o_v[:, hh * E:(hh + 1) * E] = o
        wo = pltpu.bitcast(wo_v[...], bf16)
        res = jnp.dot(o_v[...], wo, preferred_element_type=f32)
        st = res[M:].astype(bf16).astype(f32)
        gl = acc_v[pl.ds(r0, SEG), :].astype(bf16).astype(f32)
        gl = gl / (1.0 + jnp.exp(-gl))
        out_v[pl.ds(r0, SEG), :] = (x_v[pl.ds(r0, SEG), :].astype(f32) + st * gl).astype(bf16)
        @pl.when((s + 1) % (OB // SEG) == 0)
        def _():
            out_copy(s // (OB // SEG)).start()
        return res[:M].astype(bf16).astype(f32)
    lax.fori_loop(0, NSEG, step, mem_ref[...].astype(f32), unroll=2)
    for b in range(S // OB):
        out_copy(b).wait()


@functools.partial(jax.jit, static_argnames=("A_seg_len",))
def pallas_recurrent_scan__memory_aug_recurrent_mem_tr__glu_gated_glu__prompt_kernel(A_x, A_mem0, A_Wq, A_Wk, A_Wv, A_Wo, A_seg_len, B_x, B_w_gate, B_w_up, B_w_down):
    f32, bf16, u32 = jnp.float32, jnp.bfloat16, jnp.uint32
    hbm = pl.BlockSpec(memory_space=pl.ANY)
    vm = pl.BlockSpec(memory_space=pltpu.VMEM)
    V = pltpu.VMEM
    out = pl.pallas_call(
        kernel,
        out_shape=jax.ShapeDtypeStruct((S, D), bf16),
        in_specs=[hbm, vm, hbm, hbm, hbm, hbm, hbm, hbm, hbm],
        out_specs=hbm,
        scratch_shapes=[
            V((S, D), bf16), V((S // 2, D), u32), V((S, D), f32), V((S, D), bf16),
            V((D // 2, 3 * H * E), u32), V((H * E // 2, D), u32),
            V((3, 3, PD, H, E), bf16), V((3, H // NP * E, D), bf16),
            V((2, D, 2 * FC), bf16), V((8, 128), bf16), V((2, FC, D), bf16),
            V((L, H * E), f32),
            pltpu.SemaphoreType.DMA((8,)), pltpu.SemaphoreType.DMA((2, 3)),
            pltpu.SemaphoreType.DMA((3, 4)), pltpu.SemaphoreType.DMA((S // 256,)),
        ],
        compiler_params=pltpu.CompilerParams(vmem_limit_bytes=110 * 1024 * 1024),
    )(A_x.reshape(S, D), A_mem0.reshape(M, D), A_Wq, A_Wk, A_Wv, A_Wo.reshape(H * E, D), B_w_gate, B_w_up, B_w_down)
    return out.reshape(1, S, D)
```
